```python
import os as _os
_os.environ.setdefault("JAX_PLATFORMS", "cpu")
import jax
import jax.numpy as jnp

def _softmax(x, axis=-1):
    return jax.nn.softmax(x, axis=axis)
def _gelu(x):
    return jax.nn.gelu(x, approximate=True)
def _silu(x):
    return jax.nn.silu(x)
def _sigmoid(x):
    return jax.nn.sigmoid(x)
def _layernorm(x, axis=-1, eps=1e-5):
    m = jnp.mean(x, axis=axis, keepdims=True)
    v = jnp.var(x, axis=axis, keepdims=True)
    return (x - m) / jnp.sqrt(v + eps)
def _scatter_add(tgt, idx, src, axis=0):
    return tgt.at[idx].add(src)
def _segment_sum(src, seg, n):
    return jax.ops.segment_sum(src, seg, n)
class _Rng:
    def __init__(self, key):
        self._k = key
    def _next(self):
        self._k, sub = jax.random.split(self._k)
        return sub
    def normal(self, shape):
        return jax.random.normal(self._next(), shape, dtype=jnp.bfloat16)
    def randint(self, lo, hi, shape):
        return jax.random.randint(self._next(), shape, lo, hi, dtype=jnp.int32)
    def uniform(self, shape, lo=0.0, hi=1.0):
        return jax.random.uniform(self._next(), shape, jnp.bfloat16, lo, hi)
    def permutation(self, n):
        return jax.random.permutation(self._next(), n)


kernel_name = 'gated_mix__spectral_gfnet__dense_activation_silu__prompt'

def setup_inputs():
    _rng = _Rng(jax.random.key(int.from_bytes(__import__("os").urandom(4), "little")))
    _w = (lambda a: (lambda t: t.astype(jnp.bfloat16) if jnp.issubdtype(t.dtype, jnp.floating) else t)(jnp.asarray(a)))
    def _A_setup():
        B, S, D = 1, 2048, 512
        Df = D // 2 + 1
        return {
            "x": _w((lambda *s: _rng.normal(s) * 0.05)(B, S, D)),
            "w_r": _w((lambda *s: _rng.normal(s) * 0.05)(S, Df) * 0.02),
            "w_i": _w((lambda *s: _rng.normal(s) * 0.05)(S, Df) * 0.02),
        }
    _A_in = _A_setup()

    def _B_setup():
        B, S, D, F = 1, 2048, 512, 1376
        return {
            "x": _w((lambda *s: _rng.normal(s) * 0.05)(B, S, D)),
            "w1": _w((lambda *s: _rng.normal(s) * 0.05)(D, F) * (D ** -0.5)),
            "w2": _w((lambda *s: _rng.normal(s) * 0.05)(F, D) * (F ** -0.5)),
        }
    _B_in = _B_setup()

    return {
        "A_x": _A_in["x"],
        "A_w_r": _A_in["w_r"],
        "A_w_i": _A_in["w_i"],
        "B_x": _B_in["x"],
        "B_w1": _B_in["w1"],
        "B_w2": _B_in["w2"],
        "gate_w": _w((lambda *s: _rng.normal(s) * 0.05)(512) * 16.0),
    }

def reference(A_x, A_w_r, A_w_i, B_x, B_w1, B_w2, gate_w):
    def _A_ref(x, w_r, w_i):
        B, S, D = x.shape
        X = (lambda x, axes=(-2,-1): jnp.fft.rfft2(x.astype(jnp.float32), axes=axes))(x, axes=(-2, -1))
        W = w_r + 1j * w_i
        X = X * W
        y = (lambda x, s, axes=(-2,-1): jnp.fft.irfft2(x, s=s, axes=axes).astype(jnp.bfloat16))(X, (S, D), axes=(-2, -1))
        return y

    def _B_ref(x, w1, w2):
        h = jnp.einsum("bsd,df->bsf", x, w1)
        h = _silu(h)
        out = jnp.einsum("bsf,fd->bsd", h, w2)
        return out

    x = A_x
    g = _sigmoid((x * gate_w).sum(-1, keepdims=True))
    a = _A_ref(x, A_w_r, A_w_i)
    b = _B_ref(x, B_w1, B_w2)
    return g * a + (1 - g) * b
```

```python
import math
import jax
import jax.numpy as jnp
import numpy as np
import jax.experimental.pallas as pl
import jax.experimental.pallas.tpu as pltpu

S, D, F = 2048, 512, 1376
NT, TR = 32, 64
RB = 256
BF, F32 = jnp.bfloat16, jnp.float32


def _consts():
    d = np.arange(D)[:, None]
    l = np.arange(256)[None, :]
    ang = 2 * np.pi * ((d * l) % D) / D
    alt = (-1.0) ** np.arange(D)
    fr, fi = np.cos(ang), -np.sin(ang)
    fi[:, 0] = alt
    fd = np.concatenate([fr, fi], 1)
    gr, gi = 2 * np.cos(ang.T), -2 * np.sin(ang.T)
    gr[0, :] = 1.0
    gi[0, :] = alt
    gd = np.concatenate([gr, gi], 0) / (D * NT)
    r = np.arange(TR)
    f2 = np.zeros((NT, 128, 128))
    for kh in range(NT):
        k = kh + NT * np.arange(TR)
        a = 2 * np.pi * ((k[:, None] * r[None, :]) % S) / S
        c, s = np.cos(a), -np.sin(a)
        f2[kh] = np.block([[c, -s], [s, c]])
    g2 = np.transpose(f2, (0, 2, 1)) / TR
    j = np.arange(NT)
    a = 2 * np.pi * ((j[:, None] * j[None, :]) % NT) / NT
    c1 = np.zeros((128, 256))
    c2 = np.zeros((256, 128))
    for o in (0, 32):
        c1[o:o + 32, o:o + 32] = np.cos(a)
        c1[o:o + 32, 128 + o:160 + o] = -np.sin(a)
        c2[o:o + 32, o:o + 32] = np.cos(a)
        c2[128 + o:160 + o, o:o + 32] = -np.sin(a)
    a = 2 * np.pi * (r[:, None] * (np.arange(128) % 32)[None, :]) / S
    tw = np.concatenate([np.cos(a), -np.sin(a)], 0).astype(np.float32)
    b = lambda t: np.asarray(t, np.float32).astype(BF)
    return b(fd), b(gd), b(f2), b(g2), b(c1), b(c2), tw


def _fft(v, sign):
    n = len(v)
    if n == 1:
        return v
    e, o = _fft(v[0::2], sign), _fft(v[1::2], sign)
    out = [None] * n
    for k in range(n // 2):
        (er, ei), (pr, pi) = e[k], o[k]
        c, s = math.cos(2 * math.pi * k / n), sign * math.sin(2 * math.pi * k / n)
        if k == 0:
            tr, ti = pr, pi
        elif 4 * k == n:
            if sign > 0:
                out[k], out[k + n // 2] = (er - pi, ei + pr), (er + pi, ei - pr)
            else:
                out[k], out[k + n // 2] = (er + pi, ei - pr), (er - pi, ei + pr)
            continue
        elif 8 * k == n:
            tr, ti = ((pr - pi) * c, (pr + pi) * c) if sign > 0 else ((pr + pi) * c, (pi - pr) * c)
        elif 8 * k == 3 * n:
            tr, ti = ((pr + pi) * c, (pi - pr) * c) if sign > 0 else ((pr - pi) * c, (pr + pi) * c)
        else:
            tr, ti = pr * c - pi * s, pr * s + pi * c
        out[k], out[k + n // 2] = (er + tr, ei + ti), (er - tr, ei - ti)
    return out


def _dot(a, b):
    return jnp.dot(a, b, preferred_element_type=F32)


def _kernel(x_h, wr_h, wi_h, w1_h, w2_h, gw_h, fd_h, gd_h, f2_h, g2_h, c1_h, c2_h, tw_h,
            o_h,
            x, wr0, wi0, w1, w2, gw, fd, gd, f2, g2, c1, c2, tw, z, u, t, bacc, ob, sp, a0, a1, a2, b0, b1, b2, sem, osem):
    nb = S // RB
    wr, wi = (a0, a1, a2), (b0, b1, b2)
    xc = [pltpu.make_async_copy(x_h.at[pl.ds(i * RB, RB)], x.at[pl.ds(i * RB, RB)], sem.at[i])
          for i in range(nb)]
    names = [(fd_h, fd), (w1_h, w1), (w2_h, w2), (gw_h, gw), (c1_h, c1),
             (tw_h, tw), (f2_h, f2), (g2_h, g2), (c2_h, c2), (gd_h, gd)]
    cp = [pltpu.make_async_copy(a, b, sem.at[nb + i]) for i, (a, b) in enumerate(names)]
    cfd, cw1, cw2, cgw, cc1, ctw, cf2, cg2, cc2, cgd = cp
    xc[0].start()
    cfd.start()
    for c in xc[1:]:
        c.start()
    wc = [pltpu.make_async_copy(wr_h, wr0, sem.at[18]), pltpu.make_async_copy(wi_h, wi0, sem.at[19])]
    for c in cp[1:3] + wc + cp[3:]:
        c.start()

    def ffn(i):
        rows = pl.ds(pl.multiple_of(i * RB, RB), RB)
        h = _dot(x[rows, :], w1[...])
        h = h * jax.nn.sigmoid(h)
        bacc[rows, :] = _dot(h.astype(BF), w2[...])

    lane = jax.lax.broadcasted_iota(jnp.int32, (TR, 128), 1)

    cfd.wait()
    for i in range(nb):
        xc[i].wait()
        z[pl.ds(i * RB, RB), :] = _dot(x[pl.ds(i * RB, RB), :], fd[...])

    def radix_fwd(p):
        for lt in range(2):
            v = []
            for j in range(NT):
                rows = pl.ds(pl.multiple_of(j * TR + p * 8, 8), 8)
                v.append((z[rows, lt * 128:(lt + 1) * 128], z[rows, 256 + lt * 128:256 + (lt + 1) * 128]))
            v = _fft(v, -1)
            for k in range(NT):
                u[k, pl.ds(pl.multiple_of(p * 8, 8), 8), lt * 128:(lt + 1) * 128] = v[k][0]
                u[k, pl.ds(pl.multiple_of(TR + p * 8, 8), 8), lt * 128:(lt + 1) * 128] = v[k][1]

    cw1.wait()
    cw2.wait()

    def phase_b(i, c):
        ffn(i)
        for q in range(4):
            radix_fwd(i * 4 + q)
        return c
    jax.lax.fori_loop(0, 2, phase_b, 0)

    for c in (*wc, cc1, ctw, cf2, cg2, cc2):
        c.wait()
    for s_, d_ in ((wr0, wr), (wi0, wi)):
        d_[0][...] = pltpu.bitcast(s_[:, 0:128], jnp.uint32)
        d_[1][...] = pltpu.bitcast(s_[:, 128:256], jnp.uint32)
        d_[2][...] = pltpu.bitcast(jnp.broadcast_to(s_[:, 256:257].astype(F32), (S, 128)).astype(BF), jnp.uint32)
    wru, wiu = wr, wi

    def wpair(ref, m, lo):
        ref = ref[lo // 128]
        w = ref[pl.ds(m, TR, stride=NT // 2), :]
        return (pltpu.bitcast(w << 16, F32), pltpu.bitcast(w & jnp.uint32(0xFFFF0000), F32))

    p = jnp.zeros((TR, 128), F32)
    for j in range(NT):
        a = z[j * TR:(j + 1) * TR, 0:128]
        b = z[j * TR:(j + 1) * TR, 256:384]
        p = jnp.where(lane == j, pltpu.roll(a, j, 1) if j else a, p)
        p = jnp.where(lane == 32 + j, pltpu.roll(b, 32 + j, 1), p)
    uu = _dot(p.astype(BF), c1[...])
    ur, ui = uu[:, :128], uu[:, 128:]
    twr, twi = tw[0:TR, :], tw[TR:, :]
    us = jnp.concatenate([ur * twr - ui * twi, ur * twi + ui * twr], 0)
    zs = _dot(f2[0], us.astype(BF))
    sp[0:128, :] = zs
    sp[128:256, :] = jnp.zeros((128, 128), F32)

    def mid(m):
        wa = [wpair(wru, m, lo) for lo in (0, 128)]
        wb = [wpair(wiu, m, lo) for lo in (0, 128)]
        na, nb_ = wpair(wru, m, 256), wpair(wiu, m, 256)
        sr, si = sp[128:192, :], sp[192:256, :]
        for e in range(2):
            k = 2 * m + e
            zz = _dot(f2[k], u[k].astype(BF))
            zr, zi = zz[:TR], zz[TR:]
            a = jnp.concatenate([wa[0][e], wa[1][e]], 1)
            b = jnp.concatenate([wb[0][e], wb[1][e]], 1)
            y = jnp.concatenate([zr * a - zi * b, zr * b + zi * a], 0)
            u[k] = _dot(g2[k], y.astype(BF))
            sr = jnp.where(lane == k, pltpu.roll(wa[0][e], k, 1), sr)
            si = jnp.where(lane == k, pltpu.roll(wb[0][e], k, 1), si)
            sr = jnp.where(lane == 32 + k, na[e], sr)
            si = jnp.where(lane == 32 + k, nb_[e], si)
        sp[128:192, :] = sr
        sp[192:256, :] = si

    def phase_c(i, c):
        ffn(2 + i)
        for q in range(8):
            mid(i * 8 + q)
        return c
    jax.lax.fori_loop(0, 2, phase_c, 0)

    zr, zi, sr, si = sp[0:64, :], sp[64:128, :], sp[128:192, :], sp[192:256, :]
    ys = jnp.concatenate([zr * sr - zi * si, zr * si + zi * sr], 0)
    vs = _dot(g2[0], ys.astype(BF))
    vr, vi = vs[:TR], vs[TR:]
    vv = jnp.concatenate([vr * twr + vi * twi, vi * twr - vr * twi], 1)
    sp[0:TR, :] = _dot(vv.astype(BF), c2[...])

    lane8 = jax.lax.broadcasted_iota(jnp.int32, (8, 128), 1)

    def radix_inv(p):
        r0 = pl.ds(pl.multiple_of(p * 8, 8), 8)
        r1 = pl.ds(pl.multiple_of(TR + p * 8, 8), 8)
        ps = sp[r0, :]
        for lt in range(2):
            ls = slice(lt * 128, (lt + 1) * 128)
            v = _fft([(u[k, r0, ls], u[k, r1, ls]) for k in range(NT)], 1)
            for j in range(NT):
                a, b = v[j]
                if lt == 0:
                    a = jnp.where(lane8 == 0, pltpu.roll(ps, 128 - j, 1) if j else ps, a)
                    b = jnp.where(lane8 == 0, pltpu.roll(ps, 96 - j, 1), b)
                rows = pl.ds(pl.multiple_of(j * TR + p * 8, 8), 8)
                z[rows, ls] = a
                z[rows, 256 + lt * 128:256 + (lt + 1) * 128] = b

    def phase_d(i, c):
        ffn(4 + i)
        for q in range(4):
            radix_inv(i * 4 + q)
        return c
    jax.lax.fori_loop(0, 2, phase_d, 0)

    cgd.wait()
    cgw.wait()

    def fin(i):
        rows = pl.ds(i * RB, RB)
        a = _dot(z[rows, :].astype(BF), gd[...])
        g = jax.nn.sigmoid(jnp.sum(x[rows, :].astype(F32) * gw[...].astype(F32), -1, keepdims=True))
        b = bacc[rows, :]
        ob[rows, :] = (b + g * (a - b)).astype(BF)
        c = pltpu.make_async_copy(ob.at[rows], o_h.at[rows], osem.at[i])
        c.start()
        return c

    oc = []
    ffn(6)
    for i in range(3):
        oc.append(fin(i))
    ffn(7)
    for i in range(3, nb):
        oc.append(fin(i))
    for c in oc:
        c.wait()


@jax.jit
def pallas_gated_mix__spectral_gfnet__dense_activation_silu__prompt_kernel(
        A_x, A_w_r, A_w_i, B_x, B_w1, B_w2, gate_w):
    del B_x
    cs = _consts()
    ins = [A_x.reshape(S, D), A_w_r, A_w_i, B_w1, B_w2, gate_w.reshape(1, D)]
    V = pltpu.VMEM
    scratch = [V(a.shape, a.dtype) for a in ins] + [V(c.shape, c.dtype) for c in cs] + [
        V((S, D), F32), V((NT, 128, 256), F32), V((8, 128), F32), V((S, D), F32), V((S, D), BF),
        V((256, 128), F32), *[V((S // 2, 128), jnp.uint32)] * 6, pltpu.SemaphoreType.DMA((24,)), pltpu.SemaphoreType.DMA((8,))]
    out = pl.pallas_call(
        _kernel,
        out_shape=jax.ShapeDtypeStruct((S, D), BF),
        in_specs=[pl.BlockSpec(memory_space=pl.ANY)] * 13,
        out_specs=pl.BlockSpec(memory_space=pl.ANY),
        scratch_shapes=scratch,
        compiler_params=pltpu.CompilerParams(vmem_limit_bytes=100 * 1024 * 1024),
    )(*ins, *cs)
    return out.reshape(1, S, D)
```

```python
import math
import jax
import jax.numpy as jnp
import numpy as np
import jax.experimental.pallas as pl
import jax.experimental.pallas.tpu as pltpu

S, D, F = 2048, 512, 1376
NT, TR = 32, 64
RB = 256
BF, F32 = jnp.bfloat16, jnp.float32


def _consts():
    d = np.arange(256)[:, None]
    fd, gd = np.zeros((2, 256, 256)), np.zeros((2, 256, 256))
    for e in range(2):
        ang = 2 * np.pi * ((d * (2 * np.arange(128)[None, :] + e)) % D) / D
        fr, fi = np.cos(ang), -np.sin(ang)
        gr, gi = 2 * fr.T, 2 * fi.T
        if e == 0:
            fi[:, 0] = gi[0, :] = (-1.0) ** np.arange(256)
            gr[0, :] = 1.0
        fd[e] = np.concatenate([fr, fi], 1)
        gd[e] = np.concatenate([gr, gi], 0) / (D * NT)
    r = np.arange(TR)
    f2 = np.zeros((NT, 128, 128))
    for kh in range(NT):
        k = kh + NT * np.arange(TR)
        a = 2 * np.pi * ((k[:, None] * r[None, :]) % S) / S
        c, s = np.cos(a), -np.sin(a)
        f2[kh] = np.block([[c, -s], [s, c]])
    g2 = np.transpose(f2, (0, 2, 1)) / TR
    j = np.arange(NT)
    a = 2 * np.pi * ((j[:, None] * j[None, :]) % NT) / NT
    c1 = np.zeros((128, 256))
    c2 = np.zeros((256, 128))
    for o in (0, 32):
        c1[o:o + 32, o:o + 32] = np.cos(a)
        c1[o:o + 32, 128 + o:160 + o] = -np.sin(a)
        c2[o:o + 32, o:o + 32] = np.cos(a)
        c2[128 + o:160 + o, o:o + 32] = -np.sin(a)
    a = 2 * np.pi * (r[:, None] * (np.arange(128) % 32)[None, :]) / S
    tw = np.concatenate([np.cos(a), -np.sin(a)], 0).astype(np.float32)
    b = lambda t: np.asarray(t, np.float32).astype(BF)
    return b(fd), b(gd), b(f2), b(g2), b(c1), b(c2), tw


def _fft(v, sign):
    n = len(v)
    if n == 1:
        return v
    e, o = _fft(v[0::2], sign), _fft(v[1::2], sign)
    out = [None] * n
    for k in range(n // 2):
        (er, ei), (pr, pi) = e[k], o[k]
        c, s = math.cos(2 * math.pi * k / n), sign * math.sin(2 * math.pi * k / n)
        if k == 0:
            tr, ti = pr, pi
        elif 4 * k == n:
            if sign > 0:
                out[k], out[k + n // 2] = (er - pi, ei + pr), (er + pi, ei - pr)
            else:
                out[k], out[k + n // 2] = (er + pi, ei - pr), (er - pi, ei + pr)
            continue
        elif 8 * k == n:
            tr, ti = ((pr - pi) * c, (pr + pi) * c) if sign > 0 else ((pr + pi) * c, (pi - pr) * c)
        elif 8 * k == 3 * n:
            tr, ti = ((pr + pi) * c, (pi - pr) * c) if sign > 0 else ((pr - pi) * c, (pr + pi) * c)
        else:
            tr, ti = pr * c - pi * s, pr * s + pi * c
        out[k], out[k + n // 2] = (er + tr, ei + ti), (er - tr, ei - ti)
    return out


def _dot(a, b):
    return jnp.dot(a, b, preferred_element_type=F32)


def _kernel(x_h, wr_h, wi_h, w1_h, w2_h, gw_h, fd_h, gd_h, f2_h, g2_h, c1_h, c2_h, tw_h,
            o_h,
            x, wr0, wi0, w1, w2, gw, fd, gd, f2, g2, c1, c2, tw, z, u, t, bacc, ob, sp, a0, a1, a2, b0, b1, b2, sem, osem):
    nb = S // RB
    wr, wi = (a0, a1, a2), (b0, b1, b2)
    xc = [pltpu.make_async_copy(x_h.at[pl.ds(i * RB, RB)], x.at[pl.ds(i * RB, RB)], sem.at[i])
          for i in range(nb)]
    names = [(fd_h, fd), (w1_h, w1), (w2_h, w2), (gw_h, gw), (c1_h, c1),
             (tw_h, tw), (f2_h, f2), (g2_h, g2), (c2_h, c2), (gd_h, gd)]
    cp = [pltpu.make_async_copy(a, b, sem.at[nb + i]) for i, (a, b) in enumerate(names)]
    cfd, cw1, cw2, cgw, cc1, ctw, cf2, cg2, cc2, cgd = cp
    xc[0].start()
    cfd.start()
    for c in xc[1:]:
        c.start()
    wc = [pltpu.make_async_copy(wr_h, wr0, sem.at[18]), pltpu.make_async_copy(wi_h, wi0, sem.at[19])]
    for c in cp[1:3] + wc + cp[3:]:
        c.start()

    def ffn(i):
        rows = pl.ds(pl.multiple_of(i * RB, RB), RB)
        h = jax.lax.dot_general(x[rows, :], w1[...], (((1,), (1,)), ((), ())), preferred_element_type=F32)
        h = h * jax.nn.sigmoid(h)
        bacc[rows, :] = _dot(h.astype(BF), w2[...])

    lane = jax.lax.broadcasted_iota(jnp.int32, (TR, 128), 1)

    cfd.wait()
    for i in range(nb):
        xc[i].wait()
        rows = pl.ds(i * RB, RB)
        xa, xb = x[rows, 0:256].astype(F32), x[rows, 256:512].astype(F32)
        for e, v in enumerate((xa + xb, xa - xb)):
            zz = _dot(v.astype(BF), fd[e])
            z[rows, e * 128:(e + 1) * 128] = zz[:, :128]
            z[rows, 256 + e * 128:256 + (e + 1) * 128] = zz[:, 128:]

    def radix_fwd(p):
        for lt in range(2):
            v = []
            for j in range(NT):
                rows = pl.ds(pl.multiple_of(j * TR + p * 8, 8), 8)
                v.append((z[rows, lt * 128:(lt + 1) * 128], z[rows, 256 + lt * 128:256 + (lt + 1) * 128]))
            v = _fft(v, -1)
            for k in range(NT):
                u[k, pl.ds(pl.multiple_of(p * 8, 8), 8), lt * 128:(lt + 1) * 128] = v[k][0]
                u[k, pl.ds(pl.multiple_of(TR + p * 8, 8), 8), lt * 128:(lt + 1) * 128] = v[k][1]

    cw1.wait()
    cw2.wait()

    def phase_b(i, c):
        ffn(i)
        for q in range(4):
            radix_fwd(i * 4 + q)
        return c
    jax.lax.fori_loop(0, 2, phase_b, 0)

    for c in (*wc, cc1, ctw, cf2, cg2, cc2):
        c.wait()
    for s_, d_ in ((wr0, wr), (wi0, wi)):
        for q in range(S // 128):
            cs = slice(q * 128, (q + 1) * 128)
            w = pltpu.bitcast(s_[0:256, cs], jnp.uint32)
            d_[0][cs, :] = pltpu.bitcast(w << 16, F32).T
            d_[1][cs, :] = pltpu.bitcast(w & jnp.uint32(0xFFFF0000), F32).T
            d_[2][cs, :] = jnp.broadcast_to(s_[256:257, cs].astype(F32), (128, 128)).T
    wru, wiu = wr, wi

    def wpair(ref, m, lo):
        return [ref[lo // 128][pl.ds(2 * m + e, TR, stride=NT), :] for e in range(2)]

    p = jnp.zeros((TR, 128), F32)
    for j in range(NT):
        a = z[j * TR:(j + 1) * TR, 0:128]
        b = z[j * TR:(j + 1) * TR, 256:384]
        p = jnp.where(lane == j, pltpu.roll(a, j, 1) if j else a, p)
        p = jnp.where(lane == 32 + j, pltpu.roll(b, 32 + j, 1), p)
    uu = _dot(p.astype(BF), c1[...])
    ur, ui = uu[:, :128], uu[:, 128:]
    twr, twi = tw[0:TR, :], tw[TR:, :]
    us = jnp.concatenate([ur * twr - ui * twi, ur * twi + ui * twr], 0)
    zs = _dot(f2[0], us.astype(BF))
    sp[0:128, :] = zs
    sp[128:256, :] = jnp.zeros((128, 128), F32)

    def mid(m):
        wa = [wpair(wru, m, lo) for lo in (0, 128)]
        wb = [wpair(wiu, m, lo) for lo in (0, 128)]
        na, nb_ = wpair(wru, m, 256), wpair(wiu, m, 256)
        sr, si = sp[128:192, :], sp[192:256, :]
        for e in range(2):
            k = 2 * m + e
            zz = _dot(f2[k], u[k].astype(BF))
            zr, zi = zz[:TR], zz[TR:]
            a = jnp.concatenate([wa[0][e], wa[1][e]], 1)
            b = jnp.concatenate([wb[0][e], wb[1][e]], 1)
            y = jnp.concatenate([zr * a - zi * b, zr * b + zi * a], 0)
            u[k] = _dot(g2[k], y.astype(BF))
            sr = jnp.where(lane == k, pltpu.roll(wa[0][e], k, 1), sr)
            si = jnp.where(lane == k, pltpu.roll(wb[0][e], k, 1), si)
            sr = jnp.where(lane == 32 + k, na[e], sr)
            si = jnp.where(lane == 32 + k, nb_[e], si)
        sp[128:192, :] = sr
        sp[192:256, :] = si

    def phase_c(i, c):
        ffn(2 + i)
        for q in range(8):
            mid(i * 8 + q)
        return c
    jax.lax.fori_loop(0, 2, phase_c, 0)

    zr, zi, sr, si = sp[0:64, :], sp[64:128, :], sp[128:192, :], sp[192:256, :]
    ys = jnp.concatenate([zr * sr - zi * si, zr * si + zi * sr], 0)
    vs = _dot(g2[0], ys.astype(BF))
    vr, vi = vs[:TR], vs[TR:]
    vv = jnp.concatenate([vr * twr + vi * twi, vi * twr - vr * twi], 1)
    sp[0:TR, :] = _dot(vv.astype(BF), c2[...])

    lane8 = jax.lax.broadcasted_iota(jnp.int32, (8, 128), 1)

    def radix_inv(p):
        r0 = pl.ds(pl.multiple_of(p * 8, 8), 8)
        r1 = pl.ds(pl.multiple_of(TR + p * 8, 8), 8)
        ps = sp[r0, :]
        for lt in range(2):
            ls = slice(lt * 128, (lt + 1) * 128)
            v = _fft([(u[k, r0, ls], u[k, r1, ls]) for k in range(NT)], 1)
            for j in range(NT):
                a, b = v[j]
                if lt == 0:
                    a = jnp.where(lane8 == 0, pltpu.roll(ps, 128 - j, 1) if j else ps, a)
                    b = jnp.where(lane8 == 0, pltpu.roll(ps, 96 - j, 1), b)
                rows = pl.ds(pl.multiple_of(j * TR + p * 8, 8), 8)
                z[rows, ls] = a
                z[rows, 256 + lt * 128:256 + (lt + 1) * 128] = b

    def phase_d(i, c):
        ffn(4 + i)
        for q in range(4):
            radix_inv(i * 4 + q)
        return c
    jax.lax.fori_loop(0, 2, phase_d, 0)

    cgd.wait()
    cgw.wait()

    def fin(i):
        rows = pl.ds(i * RB, RB)
        ae, ao = [_dot(jnp.concatenate([z[rows, e * 128:(e + 1) * 128], z[rows, 256 + e * 128:384 + e * 128]],
                                       1).astype(BF), gd[e]) for e in range(2)]
        a = jnp.concatenate([ae + ao, ae - ao], 1)
        g = jax.nn.sigmoid(jnp.sum(x[rows, :].astype(F32) * gw[...].astype(F32), -1, keepdims=True))
        b = bacc[rows, :]
        ob[rows, :] = (b + g * (a - b)).astype(BF)
        c = pltpu.make_async_copy(ob.at[rows], o_h.at[rows], osem.at[i])
        c.start()
        return c

    oc = []
    ffn(6)
    for i in range(3):
        oc.append(fin(i))
    ffn(7)
    for i in range(3, nb):
        oc.append(fin(i))
    for c in oc:
        c.wait()


@jax.jit
def pallas_gated_mix__spectral_gfnet__dense_activation_silu__prompt_kernel(
        A_x, A_w_r, A_w_i, B_x, B_w1, B_w2, gate_w):
    del B_x
    cs = _consts()
    ins = [A_x.reshape(S, D), A_w_r.T, A_w_i.T, B_w1.T, B_w2, gate_w.reshape(1, D)]
    V = pltpu.VMEM
    scratch = [V(a.shape, a.dtype) for a in ins] + [V(c.shape, c.dtype) for c in cs] + [
        V((S, D), F32), V((NT, 128, 256), F32), V((8, 128), F32), V((S, D), F32), V((S, D), BF),
        V((256, 128), F32), *[V((S, 128), F32)] * 6, pltpu.SemaphoreType.DMA((24,)), pltpu.SemaphoreType.DMA((8,))]
    out = pl.pallas_call(
        _kernel,
        out_shape=jax.ShapeDtypeStruct((S, D), BF),
        in_specs=[pl.BlockSpec(memory_space=pltpu.HBM)] * 13,
        out_specs=pl.BlockSpec(memory_space=pltpu.HBM),
        scratch_shapes=scratch,
        compiler_params=pltpu.CompilerParams(vmem_limit_bytes=100 * 1024 * 1024),
    )(*ins, *cs)
    return out.reshape(1, S, D)
```

```python
import math
import jax
import jax.numpy as jnp
import numpy as np
import jax.experimental.pallas as pl
import jax.experimental.pallas.tpu as pltpu

S, D, F = 2048, 512, 1376
NT, TR = 32, 64
RB = 256
BF, F32 = jnp.bfloat16, jnp.float32


def _consts():
    d = np.arange(256)[:, None]
    fd, gd = np.zeros((2, 256, 256)), np.zeros((2, 256, 256))
    for e in range(2):
        ang = 2 * np.pi * ((d * (2 * np.arange(128)[None, :] + e)) % D) / D
        fr, fi = np.cos(ang), -np.sin(ang)
        gr, gi = 2 * fr.T, 2 * fi.T
        if e == 0:
            fi[:, 0] = gi[0, :] = (-1.0) ** np.arange(256)
            gr[0, :] = 1.0
        fd[e] = np.concatenate([fr, fi], 1)
        gd[e] = np.concatenate([gr, gi], 0) / (D * NT)
    r = np.arange(TR)
    f2 = np.zeros((NT, 128, 128))
    for kh in range(NT):
        k = kh + NT * np.arange(TR)
        a = 2 * np.pi * ((k[:, None] * r[None, :]) % S) / S
        c, s = np.cos(a), -np.sin(a)
        f2[kh] = np.block([[c, -s], [s, c]])
    g2 = np.transpose(f2, (0, 2, 1)) / TR
    j = np.arange(NT)
    a = 2 * np.pi * ((j[:, None] * j[None, :]) % NT) / NT
    c1 = np.zeros((128, 256))
    c2 = np.zeros((256, 128))
    for o in (0, 32):
        c1[o:o + 32, o:o + 32] = np.cos(a)
        c1[o:o + 32, 128 + o:160 + o] = -np.sin(a)
        c2[o:o + 32, o:o + 32] = np.cos(a)
        c2[128 + o:160 + o, o:o + 32] = -np.sin(a)
    a = 2 * np.pi * (r[:, None] * (np.arange(128) % 32)[None, :]) / S
    tw = np.concatenate([np.cos(a), -np.sin(a)], 0).astype(np.float32)
    b = lambda t: np.asarray(t, np.float32).astype(BF)
    return b(fd), b(gd), b(f2), b(g2), b(c1), b(c2), tw


def _fft(v, sign):
    n = len(v)
    if n == 1:
        return v
    e, o = _fft(v[0::2], sign), _fft(v[1::2], sign)
    out = [None] * n
    for k in range(n // 2):
        (er, ei), (pr, pi) = e[k], o[k]
        c, s = math.cos(2 * math.pi * k / n), sign * math.sin(2 * math.pi * k / n)
        if k == 0:
            tr, ti = pr, pi
        elif 4 * k == n:
            if sign > 0:
                out[k], out[k + n // 2] = (er - pi, ei + pr), (er + pi, ei - pr)
            else:
                out[k], out[k + n // 2] = (er + pi, ei - pr), (er - pi, ei + pr)
            continue
        elif 8 * k == n:
            tr, ti = ((pr - pi) * c, (pr + pi) * c) if sign > 0 else ((pr + pi) * c, (pi - pr) * c)
        elif 8 * k == 3 * n:
            tr, ti = ((pr + pi) * c, (pi - pr) * c) if sign > 0 else ((pr - pi) * c, (pr + pi) * c)
        else:
            tr, ti = pr * c - pi * s, pr * s + pi * c
        out[k], out[k + n // 2] = (er + tr, ei + ti), (er - tr, ei - ti)
    return out


def _dot(a, b):
    return jnp.dot(a, b, preferred_element_type=F32)


def _kernel(x_h, wr_h, wi_h, w1_h, w2_h, gw_h, fd_h, gd_h, f2_h, g2_h, c1_h, c2_h, tw_h,
            o_h,
            x, wr0, wi0, w1, w2, gw, fd, gd, f2, g2, c1, c2, tw, z, u, t, bacc, ob, sp, a0, a1, a2, b0, b1, b2, sem, osem):
    nb = S // RB
    wr, wi = (a0, a1, a2), (b0, b1, b2)
    xc = [pltpu.make_async_copy(x_h.at[pl.ds(i * RB, RB)], x.at[pl.ds(i * RB, RB)], sem.at[i])
          for i in range(nb)]
    names = [(fd_h, fd), (w1_h, w1), (w2_h, w2), (gw_h, gw), (c1_h, c1),
             (tw_h, tw), (f2_h, f2), (g2_h, g2), (c2_h, c2), (gd_h, gd)]
    cp = [pltpu.make_async_copy(a, b, sem.at[nb + i]) for i, (a, b) in enumerate(names)]
    cfd, cw1, cw2, cgw, cc1, ctw, cf2, cg2, cc2, cgd = cp
    xc[0].start()
    cfd.start()
    for c in xc[1:]:
        c.start()
    wc = [pltpu.make_async_copy(wr_h, wr0, sem.at[18]), pltpu.make_async_copy(wi_h, wi0, sem.at[19])]
    for c in cp[1:3] + wc + cp[3:]:
        c.start()

    def ffn(i):
        rows = pl.ds(pl.multiple_of(i * RB, RB), RB)
        h = jax.lax.dot_general(x[rows, :], w1[...], (((1,), (1,)), ((), ())), preferred_element_type=F32)
        h = 0.5 * h
        h = h + h * jnp.tanh(h)
        bacc[rows, :] = _dot(h.astype(BF), w2[...])

    lane = jax.lax.broadcasted_iota(jnp.int32, (TR, 128), 1)

    cfd.wait()
    for i in range(nb):
        xc[i].wait()
        rows = pl.ds(i * RB, RB)
        xa, xb = x[rows, 0:256].astype(F32), x[rows, 256:512].astype(F32)
        for e, v in enumerate((xa + xb, xa - xb)):
            zz = _dot(v.astype(BF), fd[e])
            z[rows, e * 128:(e + 1) * 128] = zz[:, :128]
            z[rows, 256 + e * 128:256 + (e + 1) * 128] = zz[:, 128:]

    def radix_fwd(p):
        for lt in range(2):
            v = []
            for j in range(NT):
                rows = pl.ds(pl.multiple_of(j * TR + p * 8, 8), 8)
                v.append((z[rows, lt * 128:(lt + 1) * 128], z[rows, 256 + lt * 128:256 + (lt + 1) * 128]))
            v = _fft(v, -1)
            for k in range(NT):
                u[k, pl.ds(pl.multiple_of(p * 8, 8), 8), lt * 128:(lt + 1) * 128] = v[k][0]
                u[k, pl.ds(pl.multiple_of(TR + p * 8, 8), 8), lt * 128:(lt + 1) * 128] = v[k][1]

    def wprep(q):
        cs = pl.ds(pl.multiple_of(q * 128, 128), 128)
        for s_, d_ in ((wr0, wr), (wi0, wi)):
            w = pltpu.bitcast(s_[0:256, cs], jnp.uint32)
            d_[0][cs, :] = pltpu.bitcast(w << 16, F32).T
            d_[1][cs, :] = pltpu.bitcast(w & jnp.uint32(0xFFFF0000), F32).T
            d_[2][cs, :] = jnp.broadcast_to(s_[256:257, cs].astype(F32), (128, 128)).T

    for c in wc:
        c.wait()
    cw1.wait()
    cw2.wait()

    def phase_b(i, c):
        ffn(i)
        for q in range(4):
            radix_fwd(i * 4 + q)
            wprep(i * 8 + q)
            wprep(i * 8 + 4 + q)
        return c
    jax.lax.fori_loop(0, 2, phase_b, 0)

    for c in (cc1, ctw, cf2, cg2, cc2):
        c.wait()
    wru, wiu = wr, wi

    def wpair(ref, m, lo):
        return [ref[lo // 128][pl.ds(2 * m + e, TR, stride=NT), :] for e in range(2)]

    p = jnp.zeros((TR, 128), F32)
    for j in range(NT):
        a = z[j * TR:(j + 1) * TR, 0:128]
        b = z[j * TR:(j + 1) * TR, 256:384]
        p = jnp.where(lane == j, pltpu.roll(a, j, 1) if j else a, p)
        p = jnp.where(lane == 32 + j, pltpu.roll(b, 32 + j, 1), p)
    uu = _dot(p.astype(BF), c1[...])
    ur, ui = uu[:, :128], uu[:, 128:]
    twr, twi = tw[0:TR, :], tw[TR:, :]
    us = jnp.concatenate([ur * twr - ui * twi, ur * twi + ui * twr], 0)
    zs = _dot(f2[0], us.astype(BF))
    sp[0:128, :] = zs
    sp[128:256, :] = jnp.zeros((128, 128), F32)

    def mid(m):
        wa = [wpair(wru, m, lo) for lo in (0, 128)]
        wb = [wpair(wiu, m, lo) for lo in (0, 128)]
        na, nb_ = wpair(wru, m, 256), wpair(wiu, m, 256)
        sr, si = sp[128:192, :], sp[192:256, :]
        for e in range(2):
            k = 2 * m + e
            zz = _dot(f2[k], u[k].astype(BF))
            zr, zi = zz[:TR], zz[TR:]
            a = jnp.concatenate([wa[0][e], wa[1][e]], 1)
            b = jnp.concatenate([wb[0][e], wb[1][e]], 1)
            y = jnp.concatenate([zr * a - zi * b, zr * b + zi * a], 0)
            u[k] = _dot(g2[k], y.astype(BF))
            sr = jnp.where(lane == k, pltpu.roll(wa[0][e], k, 1), sr)
            si = jnp.where(lane == k, pltpu.roll(wb[0][e], k, 1), si)
            sr = jnp.where(lane == 32 + k, na[e], sr)
            si = jnp.where(lane == 32 + k, nb_[e], si)
        sp[128:192, :] = sr
        sp[192:256, :] = si

    def phase_c(i, c):
        ffn(2 + i)
        for q in range(8):
            mid(i * 8 + q)
        return c
    jax.lax.fori_loop(0, 2, phase_c, 0)

    zr, zi, sr, si = sp[0:64, :], sp[64:128, :], sp[128:192, :], sp[192:256, :]
    ys = jnp.concatenate([zr * sr - zi * si, zr * si + zi * sr], 0)
    vs = _dot(g2[0], ys.astype(BF))
    vr, vi = vs[:TR], vs[TR:]
    vv = jnp.concatenate([vr * twr + vi * twi, vi * twr - vr * twi], 1)
    sp[0:TR, :] = _dot(vv.astype(BF), c2[...])

    lane8 = jax.lax.broadcasted_iota(jnp.int32, (8, 128), 1)

    def radix_inv(p):
        r0 = pl.ds(pl.multiple_of(p * 8, 8), 8)
        r1 = pl.ds(pl.multiple_of(TR + p * 8, 8), 8)
        ps = sp[r0, :]
        for lt in range(2):
            ls = slice(lt * 128, (lt + 1) * 128)
            v = _fft([(u[k, r0, ls], u[k, r1, ls]) for k in range(NT)], 1)
            for j in range(NT):
                a, b = v[j]
                if lt == 0:
                    a = jnp.where(lane8 == 0, pltpu.roll(ps, 128 - j, 1) if j else ps, a)
                    b = jnp.where(lane8 == 0, pltpu.roll(ps, 96 - j, 1), b)
                rows = pl.ds(pl.multiple_of(j * TR + p * 8, 8), 8)
                z[rows, ls] = a
                z[rows, 256 + lt * 128:256 + (lt + 1) * 128] = b

    def phase_d(i, c):
        ffn(4 + i)
        for q in range(4):
            radix_inv(i * 4 + q)
        return c
    jax.lax.fori_loop(0, 2, phase_d, 0)

    cgd.wait()
    cgw.wait()

    def fin(i):
        rows = pl.ds(i * RB, RB)
        ae, ao = [_dot(jnp.concatenate([z[rows, e * 128:(e + 1) * 128], z[rows, 256 + e * 128:384 + e * 128]],
                                       1).astype(BF), gd[e]) for e in range(2)]
        a = jnp.concatenate([ae + ao, ae - ao], 1)
        g = jax.nn.sigmoid(jnp.sum(x[rows, :].astype(F32) * gw[...].astype(F32).reshape(1, D), -1, keepdims=True))
        b = bacc[rows, :]
        ob[rows, :] = (b + g * (a - b)).astype(BF)
        c = pltpu.make_async_copy(ob.at[rows], o_h.at[rows], osem.at[i])
        c.start()
        return c

    oc = []
    ffn(6)
    for i in range(3):
        oc.append(fin(i))
    ffn(7)
    for i in range(3, nb):
        oc.append(fin(i))
    for c in oc:
        c.wait()


@jax.jit
def pallas_gated_mix__spectral_gfnet__dense_activation_silu__prompt_kernel(
        A_x, A_w_r, A_w_i, B_x, B_w1, B_w2, gate_w):
    del B_x
    cs = _consts()
    ins = [A_x.reshape(S, D), A_w_r.T, A_w_i.T, B_w1.T, B_w2, gate_w]
    V = pltpu.VMEM
    scratch = [V(a.shape, a.dtype) for a in ins] + [V(c.shape, c.dtype) for c in cs] + [
        V((S, D), F32), V((NT, 128, 256), F32), V((8, 128), F32), V((S, D), F32), V((S, D), BF),
        V((256, 128), F32), *[V((S, 128), F32)] * 6, pltpu.SemaphoreType.DMA((24,)), pltpu.SemaphoreType.DMA((8,))]
    out = pl.pallas_call(
        _kernel,
        out_shape=jax.ShapeDtypeStruct((S, D), BF),
        in_specs=[pl.BlockSpec(memory_space=pltpu.HBM)] * 13,
        out_specs=pl.BlockSpec(memory_space=pltpu.HBM),
        scratch_shapes=scratch,
        compiler_params=pltpu.CompilerParams(vmem_limit_bytes=100 * 1024 * 1024),
    )(*ins, *cs)
    return out.reshape(1, S, D)
```

```python
import math
import jax
import jax.numpy as jnp
import numpy as np
import jax.experimental.pallas as pl
import jax.experimental.pallas.tpu as pltpu

S, D, F = 2048, 512, 1376
NT, TR = 32, 64
RB = 256
BF, F32 = jnp.bfloat16, jnp.float32


def _consts():
    d = np.arange(256)[:, None]
    fd, gd = np.zeros((2, 256, 256)), np.zeros((2, 256, 256))
    for e in range(2):
        ang = 2 * np.pi * ((d * (2 * np.arange(128)[None, :] + e)) % D) / D
        fr, fi = np.cos(ang), -np.sin(ang)
        gr, gi = 2 * fr.T, 2 * fi.T
        if e == 0:
            fi[:, 0] = gi[0, :] = (-1.0) ** np.arange(256)
            gr[0, :] = 1.0
        fd[e] = np.concatenate([fr, fi], 1)
        gd[e] = np.concatenate([gr, gi], 0) / (D * NT)
    r = np.arange(TR)
    f2 = np.zeros((NT, 128, 128))
    for kh in range(NT):
        k = kh + NT * np.arange(TR)
        a = 2 * np.pi * ((k[:, None] * r[None, :]) % S) / S
        c, s = np.cos(a), -np.sin(a)
        f2[kh] = np.block([[c, -s], [s, c]])
    g2 = np.transpose(f2, (0, 2, 1)) / TR
    j = np.arange(NT)
    a = 2 * np.pi * ((j[:, None] * j[None, :]) % NT) / NT
    c1 = np.zeros((128, 256))
    c2 = np.zeros((256, 128))
    for o in (0, 32):
        c1[o:o + 32, o:o + 32] = np.cos(a)
        c1[o:o + 32, 128 + o:160 + o] = -np.sin(a)
        c2[o:o + 32, o:o + 32] = np.cos(a)
        c2[128 + o:160 + o, o:o + 32] = -np.sin(a)
    a = 2 * np.pi * (r[:, None] * (np.arange(128) % 32)[None, :]) / S
    tw = np.concatenate([np.cos(a), -np.sin(a)], 0).astype(np.float32)
    b = lambda t: np.asarray(t, np.float32).astype(BF)
    return b(fd), b(gd), b(f2), b(g2), b(c1), b(c2), tw


def _fft(v, sign):
    n = len(v)
    if n == 1:
        return v
    e, o = _fft(v[0::2], sign), _fft(v[1::2], sign)
    out = [None] * n
    for k in range(n // 2):
        (er, ei), (pr, pi) = e[k], o[k]
        c, s = math.cos(2 * math.pi * k / n), sign * math.sin(2 * math.pi * k / n)
        if k == 0:
            tr, ti = pr, pi
        elif 4 * k == n:
            if sign > 0:
                out[k], out[k + n // 2] = (er - pi, ei + pr), (er + pi, ei - pr)
            else:
                out[k], out[k + n // 2] = (er + pi, ei - pr), (er - pi, ei + pr)
            continue
        elif 8 * k == n:
            tr, ti = ((pr - pi) * c, (pr + pi) * c) if sign > 0 else ((pr + pi) * c, (pi - pr) * c)
        elif 8 * k == 3 * n:
            tr, ti = ((pr + pi) * c, (pi - pr) * c) if sign > 0 else ((pr - pi) * c, (pr + pi) * c)
        else:
            tr, ti = pr * c - pi * s, pr * s + pi * c
        out[k], out[k + n // 2] = (er + tr, ei + ti), (er - tr, ei - ti)
    return out


def _mo(i, n):
    return i if isinstance(i, int) else pl.multiple_of(i, n)


def _dot(a, b):
    return jnp.dot(a, b, preferred_element_type=F32)


def _kernel(x_h, wr_h, wi_h, w1_h, w2_h, gw_h, fd_h, gd_h, f2_h, g2_h, c1_h, c2_h, tw_h,
            o_h,
            x, wr0, wi0, w1, w2, gw, fd, gd, f2, g2, c1, c2, tw, z, u, t, bacc, ob, sp, a0, a1, a2, b0, b1, b2, sem, osem):
    nb = S // RB
    wr, wi = (a0, a1, a2), (b0, b1, b2)
    xc = [pltpu.make_async_copy(x_h.at[pl.ds(i * RB, RB)], x.at[pl.ds(i * RB, RB)], sem.at[i])
          for i in range(nb)]
    names = [(fd_h, fd), (w1_h, w1), (w2_h, w2), (gw_h, gw), (c1_h, c1),
             (tw_h, tw), (f2_h, f2), (g2_h, g2), (c2_h, c2), (gd_h, gd)]
    cp = [pltpu.make_async_copy(a, b, sem.at[nb + i]) for i, (a, b) in enumerate(names)]
    cfd, cw1, cw2, cgw, cc1, ctw, cf2, cg2, cc2, cgd = cp
    xc[0].start()
    cfd.start()
    for c in xc[1:]:
        c.start()
    wc = [pltpu.make_async_copy(wr_h, wr0, sem.at[18]), pltpu.make_async_copy(wi_h, wi0, sem.at[19])]
    for c in cp[1:3]:
        c.start()

    def ffn(i):
        rows = pl.ds(_mo(i * RB, RB), RB)
        h = jax.lax.dot_general(x[rows, :], w1[...], (((1,), (1,)), ((), ())), preferred_element_type=F32)
        h = 0.5 * h
        h = h + h * jnp.tanh(h)
        bacc[rows, :] = _dot(h.astype(BF), w2[...])

    lane = jax.lax.broadcasted_iota(jnp.int32, (TR, 128), 1)

    cfd.wait()
    for i in range(nb):
        xc[i].wait()
        rows = pl.ds(i * RB, RB)
        xa, xb = x[rows, 0:256].astype(F32), x[rows, 256:512].astype(F32)
        for e, v in enumerate((xa + xb, xa - xb)):
            zz = _dot(v.astype(BF), fd[e])
            z[rows, e * 128:(e + 1) * 128] = zz[:, :128]
            z[rows, 256 + e * 128:256 + (e + 1) * 128] = zz[:, 128:]

    def radix_fwd(p):
        for lt in range(2):
            v = []
            for j in range(NT):
                rows = pl.ds(_mo(j * TR + p * 8, 8), 8)
                v.append((z[rows, lt * 128:(lt + 1) * 128], z[rows, 256 + lt * 128:256 + (lt + 1) * 128]))
            v = _fft(v, -1)
            for k in range(NT):
                u[k, pl.ds(_mo(p * 8, 8), 8), lt * 128:(lt + 1) * 128] = v[k][0]
                u[k, pl.ds(_mo(TR + p * 8, 8), 8), lt * 128:(lt + 1) * 128] = v[k][1]

    def wprep(q):
        cs = pl.ds(_mo(q * 128, 128), 128)
        for s_, d_ in ((wr0, wr), (wi0, wi)):
            w = pltpu.bitcast(s_[0:256, cs], jnp.uint32)
            d_[0][cs, :] = pltpu.bitcast(w << 16, F32).T
            d_[1][cs, :] = pltpu.bitcast(w & jnp.uint32(0xFFFF0000), F32).T
            d_[2][cs, :] = jnp.broadcast_to(s_[256:257, cs].astype(F32), (128, 128)).T

    cw1.wait()
    cw2.wait()
    for c in wc + cp[3:]:
        c.start()

    def phase_b(i, c):
        ffn(i)
        for q in range(4):
            radix_fwd(i * 4 + q)
            if i:
                for q2 in range(4):
                    wprep(q * 4 + q2)
        return c
    phase_b(0, 0)
    wc[0].wait(); wc[1].wait()
    phase_b(1, 0)

    for c in (cc1, ctw, cf2, cg2, cc2):
        c.wait()
    wru, wiu = wr, wi

    def wpair(ref, m, lo):
        return [ref[lo // 128][pl.ds(2 * m + e, TR, stride=NT), :] for e in range(2)]

    p = jnp.zeros((TR, 128), F32)
    for j in range(NT):
        a = z[j * TR:(j + 1) * TR, 0:128]
        b = z[j * TR:(j + 1) * TR, 256:384]
        p = jnp.where(lane == j, pltpu.roll(a, j, 1) if j else a, p)
        p = jnp.where(lane == 32 + j, pltpu.roll(b, 32 + j, 1), p)
    uu = _dot(p.astype(BF), c1[...])
    ur, ui = uu[:, :128], uu[:, 128:]
    twr, twi = tw[0:TR, :], tw[TR:, :]
    us = jnp.concatenate([ur * twr - ui * twi, ur * twi + ui * twr], 0)
    zs = _dot(f2[0], us.astype(BF))
    sp[0:128, :] = zs
    sp[128:256, :] = jnp.zeros((128, 128), F32)

    def mid(m):
        wa = [wpair(wru, m, lo) for lo in (0, 128)]
        wb = [wpair(wiu, m, lo) for lo in (0, 128)]
        na, nb_ = wpair(wru, m, 256), wpair(wiu, m, 256)
        sr, si = sp[128:192, :], sp[192:256, :]
        for e in range(2):
            k = 2 * m + e
            zz = _dot(f2[k], u[k].astype(BF))
            zr, zi = zz[:TR], zz[TR:]
            a = jnp.concatenate([wa[0][e], wa[1][e]], 1)
            b = jnp.concatenate([wb[0][e], wb[1][e]], 1)
            y = jnp.concatenate([zr * a - zi * b, zr * b + zi * a], 0)
            u[k] = _dot(g2[k], y.astype(BF))
            sr = jnp.where(lane == k, pltpu.roll(wa[0][e], k, 1), sr)
            si = jnp.where(lane == k, pltpu.roll(wb[0][e], k, 1), si)
            sr = jnp.where(lane == 32 + k, na[e], sr)
            si = jnp.where(lane == 32 + k, nb_[e], si)
        sp[128:192, :] = sr
        sp[192:256, :] = si

    def phase_c(i, c):
        ffn(2 + i)
        for q in range(8):
            mid(i * 8 + q)
        return c
    phase_c(0, 0); phase_c(1, 0)

    zr, zi, sr, si = sp[0:64, :], sp[64:128, :], sp[128:192, :], sp[192:256, :]
    ys = jnp.concatenate([zr * sr - zi * si, zr * si + zi * sr], 0)
    vs = _dot(g2[0], ys.astype(BF))
    vr, vi = vs[:TR], vs[TR:]
    vv = jnp.concatenate([vr * twr + vi * twi, vi * twr - vr * twi], 1)
    sp[0:TR, :] = _dot(vv.astype(BF), c2[...])

    lane8 = jax.lax.broadcasted_iota(jnp.int32, (8, 128), 1)

    def radix_inv(p):
        r0 = pl.ds(_mo(p * 8, 8), 8)
        r1 = pl.ds(_mo(TR + p * 8, 8), 8)
        ps = sp[r0, :]
        for lt in range(2):
            ls = slice(lt * 128, (lt + 1) * 128)
            v = _fft([(u[k, r0, ls], u[k, r1, ls]) for k in range(NT)], 1)
            for j in range(NT):
                a, b = v[j]
                if lt == 0:
                    a = jnp.where(lane8 == 0, pltpu.roll(ps, 128 - j, 1) if j else ps, a)
                    b = jnp.where(lane8 == 0, pltpu.roll(ps, 96 - j, 1), b)
                rows = pl.ds(_mo(j * TR + p * 8, 8), 8)
                z[rows, ls] = a
                z[rows, 256 + lt * 128:256 + (lt + 1) * 128] = b

    def phase_d(i, c):
        ffn(4 + i)
        for q in range(4):
            radix_inv(i * 4 + q)
        return c
    phase_d(0, 0); phase_d(1, 0)

    cgd.wait()
    cgw.wait()

    def fin(i):
        rows = pl.ds(i * RB, RB)
        ae, ao = [_dot(jnp.concatenate([z[rows, e * 128:(e + 1) * 128], z[rows, 256 + e * 128:384 + e * 128]],
                                       1).astype(BF), gd[e]) for e in range(2)]
        a = jnp.concatenate([ae + ao, ae - ao], 1)
        g = jax.nn.sigmoid(jnp.sum(x[rows, :].astype(F32) * gw[...].astype(F32).reshape(1, D), -1, keepdims=True))
        b = bacc[rows, :]
        ob[rows, :] = (b + g * (a - b)).astype(BF)
        c = pltpu.make_async_copy(ob.at[rows], o_h.at[rows], osem.at[i])
        c.start()
        return c

    oc = []
    ffn(6)
    for i in range(6):
        oc.append(fin(i))
    ffn(7)
    for i in range(6, nb):
        oc.append(fin(i))
    for c in oc:
        c.wait()


@jax.jit
def pallas_gated_mix__spectral_gfnet__dense_activation_silu__prompt_kernel(
        A_x, A_w_r, A_w_i, B_x, B_w1, B_w2, gate_w):
    del B_x
    cs = _consts()
    ins = [A_x.reshape(S, D), A_w_r.T, A_w_i.T, B_w1.T, B_w2, gate_w]
    V = pltpu.VMEM
    scratch = [V(a.shape, a.dtype) for a in ins] + [V(c.shape, c.dtype) for c in cs] + [
        V((S, D), F32), V((NT, 128, 256), F32), V((8, 128), F32), V((S, D), F32), V((S, D), BF),
        V((256, 128), F32), *[V((S, 128), F32)] * 6, pltpu.SemaphoreType.DMA((24,)), pltpu.SemaphoreType.DMA((8,))]
    out = pl.pallas_call(
        _kernel,
        out_shape=jax.ShapeDtypeStruct((S, D), BF),
        in_specs=[pl.BlockSpec(memory_space=pltpu.HBM)] * 13,
        out_specs=pl.BlockSpec(memory_space=pltpu.HBM),
        scratch_shapes=scratch,
        compiler_params=pltpu.CompilerParams(vmem_limit_bytes=100 * 1024 * 1024),
    )(*ins, *cs)
    return out.reshape(1, S, D)
```
